```python
import os as _os
_os.environ.setdefault("JAX_PLATFORMS", "cpu")
import jax
import jax.numpy as jnp

def _softmax(x, axis=-1):
    return jax.nn.softmax(x, axis=axis)
def _gelu(x):
    return jax.nn.gelu(x, approximate=True)
def _silu(x):
    return jax.nn.silu(x)
def _sigmoid(x):
    return jax.nn.sigmoid(x)
def _layernorm(x, axis=-1, eps=1e-5):
    m = jnp.mean(x, axis=axis, keepdims=True)
    v = jnp.var(x, axis=axis, keepdims=True)
    return (x - m) / jnp.sqrt(v + eps)
def _scatter_add(tgt, idx, src, axis=0):
    return tgt.at[idx].add(src)
def _segment_sum(src, seg, n):
    return jax.ops.segment_sum(src, seg, n)
class _Rng:
    def __init__(self, key):
        self._k = key
    def _next(self):
        self._k, sub = jax.random.split(self._k)
        return sub
    def normal(self, shape):
        return jax.random.normal(self._next(), shape, dtype=jnp.bfloat16)
    def randint(self, lo, hi, shape):
        return jax.random.randint(self._next(), shape, lo, hi, dtype=jnp.int32)
    def uniform(self, shape, lo=0.0, hi=1.0):
        return jax.random.uniform(self._next(), shape, jnp.bfloat16, lo, hi)
    def permutation(self, n):
        return jax.random.permutation(self._next(), n)


kernel_name = 'standalone__gqa_block_cached__near_ridge'

def setup_inputs():
    _rng = _Rng(jax.random.key(int.from_bytes(__import__("os").urandom(4), "little")))
    _w = (lambda a: (lambda t: t.astype(jnp.bfloat16) if jnp.issubdtype(t.dtype, jnp.floating) else t)(jnp.asarray(a)))
    B, Sq, D = 16, 128, 576
    Hq, Hkv, Sk, Dh = 32, 16, 1024, 128
    assert Hq % Hkv == 0, (Hq, Hkv)
    return {
        "x": _w((lambda *s: _rng.normal(s) * 0.8)(B, Sq, D)),
        "k_cache": _w((lambda *s: _rng.normal(s) * 0.8)(B, Hkv, Sk, Dh)),
        "v_cache": _w((lambda *s: _rng.normal(s) * 0.05)(B, Hkv, Sk, Dh)),
        "wq": _w((lambda *s: _rng.normal(s) * 0.8)(D, Hq * Dh) * (D ** -0.5)),
        "wo": _w((lambda *s: _rng.normal(s) * 0.05)(Hq * Dh, D) * ((Hq * Dh) ** -0.5)),
    }

def reference(x, k_cache, v_cache, wq, wo):
    B, Sq, D = x.shape
    Hq, Dh = 32, 128
    Hkv = k_cache.shape[1]
    rep = Hq // Hkv
    q = (lambda x, *d: x.transpose(*d))((x @ wq).reshape(B, Sq, Hq, Dh), 0, 2, 1, 3)
    k = jnp.repeat(k_cache, rep, axis=1)
    v = jnp.repeat(v_cache, rep, axis=1)
    scores = jnp.einsum("bhqd,bhkd->bhqk", q, k) * (Dh ** -0.5)
    p = _softmax(scores, axis=-1)
    o = jnp.einsum("bhqk,bhkd->bhqd", p, v)
    return (lambda x, *d: x.transpose(*d))(o, 0, 2, 1, 3).reshape(B, Sq, Hq * Dh) @ wo
```

```python
import functools
import os
import jax
import jax.numpy as jnp
import jax.experimental.pallas as pl
import jax.experimental.pallas.tpu as pltpu

LOG2E = 1.4426950408889634
NP = 4
ORDER = os.environ.get("ORDER", "C0 B B C1 B A0 B A1 B Q B B B D")
NB = int(os.environ.get("NB", "8"))
UNROLL = int(os.environ.get("UNROLL", "1"))
FLAGS = {k: True for k in os.environ.get("KFLAGS", "XLA_TPU_EVENLY_DISTRIBUTE_CRITICAL_NODES").split() if k}


class _Multi:
    def __init__(self, copies):
        self.copies = copies

    def start(self):
        for c in self.copies:
            c.start()

    def wait(self):
        for c in self.copies:
            c.wait()


def _kernel(xT_hbm, k_hbm, v_hbm, wq_hbm, woT_hbm, outT_hbm,
            xT_v, x_scr, wq_v, wo_v, k_buf, v_buf,
            q0, q1, s0, s1, m0, m1, p0, p1, l0, l1, opart, acc, ostage,
            sem_x, sem_w, sem_k, sem_v, sem_o, *, scale):
    B, D, Sq = xT_hbm.shape
    _, GP, _, Sk, Dh = k_hbm.shape
    n_pairs = B * GP
    n_units = 2 * n_pairs
    LB = B.bit_length() - 1
    assert B == 1 << LB
    f32, bf16, u32 = jnp.float32, jnp.bfloat16, jnp.uint32
    qs, ss, ms, ps, ls = (q0, q1), (s0, s1), (m0, m1), (p0, p1), (l0, l1)
    R = 2 * Sq
    NC = Sk // Dh
    HK = Sk // 2

    def batch_of(u):
        return (u >> 1) & (B - 1)

    def kvhead_of(u):
        return ((u >> (LB + 1)) << 1) | (u & 1)

    def k_copy(p):
        s = p & (NP - 1)
        pc = jnp.minimum(p, n_pairs - 1)
        return pltpu.make_async_copy(k_hbm.at[pc & (B - 1), pc >> LB], k_buf.at[s], sem_k.at[s])

    def v_copy(p):
        s = p & (NP - 1)
        pc = jnp.minimum(p, n_pairs - 1)
        return pltpu.make_async_copy(v_hbm.at[pc & (B - 1), pc >> LB], v_buf.at[s], sem_v.at[s])

    def w_copy(src, dst, which, h0, n):
        return _Multi([pltpu.make_async_copy(src.at[:, pl.ds(pl.multiple_of((h0 + i) * Dh, Dh), Dh)],
                                             dst.at[h0 + i], sem_w.at[which]) for i in range(n)])

    def x_copy(b, n=1):
        return pltpu.make_async_copy(xT_hbm.at[pl.ds(b, n)], xT_v.at[pl.ds(b, n)], sem_x.at[b & 3])

    def o_copy(b):
        return pltpu.make_async_copy(ostage.at[b], outT_hbm.at[b], sem_o.at[0])

    def unpack(w):
        return pltpu.bitcast(w, bf16)

    def pack(v):
        return pltpu.bitcast(v, u32)

    def stage_X(b):
        x_scr[b] = pack(unpack(xT_v.bitcast(u32)[b]).T)

    def stage_Q(u, slot):
        g = kvhead_of(u)
        x = unpack(x_scr[batch_of(u)])
        wu = wq_v.bitcast(u32)
        w = jnp.concatenate([unpack(wu[2 * g]), unpack(wu[2 * g + 1])], axis=1)
        q = (jnp.dot(x, w, preferred_element_type=f32) * scale).astype(bf16)
        qs[slot][:Sq // 2, :] = pack(q[:, :Dh])
        qs[slot][Sq // 2:, :] = pack(q[:, Dh:])

    def stage_A(u, slot, h):
        k = unpack(k_buf.bitcast(u32)[(u >> 1) & (NP - 1), slot, h * (HK // 2):(h + 1) * (HK // 2), :])
        s = jax.lax.dot_general(unpack(qs[slot][...]), k, (((1,), (1,)), ((), ())),
                                preferred_element_type=f32)
        ss[slot][:, h * HK:(h + 1) * HK] = s
        mx = s[:, :Dh]
        for c in range(1, HK // Dh):
            mx = jnp.maximum(mx, s[:, c * Dh:(c + 1) * Dh])
        if h == 0:
            ms[slot][...] = mx
        else:
            mx = jnp.maximum(mx, ms[slot][...])
            ms[slot][...] = jnp.broadcast_to(jnp.max(mx, axis=-1, keepdims=True), (R, Dh))

    def stage_B(slot, i, n):
        rc = R // n
        rows = slice(i * rc, (i + 1) * rc)
        m = ms[slot][rows, :]
        p = jnp.exp2(ss[slot][rows, :] - jnp.concatenate([m] * NC, axis=1))
        l = p[:, :Dh]
        for c in range(1, NC):
            l = l + p[:, c * Dh:(c + 1) * Dh]
        l = jnp.sum(l, axis=-1, keepdims=True)
        ls[slot][rows, :] = jnp.broadcast_to(pl.reciprocal(l, approx=True), (rc, Dh))
        ps[slot][i * (rc // 2):(i + 1) * (rc // 2), :] = pack(p.astype(bf16))

    def stage_C(u, slot, h):
        v = unpack(v_buf.bitcast(u32)[(u >> 1) & (NP - 1), slot, h * (HK // 2):(h + 1) * (HK // 2), :])
        o = jnp.dot(unpack(ps[slot][:, h * HK:(h + 1) * HK]), v, preferred_element_type=f32)
        if h == 0:
            opart[...] = o
            return None
        return ((opart[...] + o) * ls[slot][...]).astype(bf16)

    def stage_D(u, o):
        g = kvhead_of(u)
        b = batch_of(u)
        o2 = jnp.concatenate([o[:Sq], o[Sq:]], axis=1)
        wo_u = wo_v.bitcast(u32)
        w2 = jnp.concatenate([unpack(wo_u[2 * g]), unpack(wo_u[2 * g + 1])], axis=1)
        c = jax.lax.dot_general(w2, o2, (((1,), (1,)), ((), ())), preferred_element_type=f32)
        acc[b] += c

    def step(uQ=None, uA=None, B_slot=None, uC=None, sQ=0, sA=0, sC=0):
        todo = list(range(NB)) if B_slot is not None else []
        o = None
        for tok in ORDER.split():
            if tok == "B":
                if todo:
                    stage_B(B_slot, todo.pop(0), NB)
            elif tok == "Q":
                if uQ is not None:
                    stage_Q(uQ, sQ)
            elif tok[0] == "C" and uC is not None:
                o = stage_C(uC, sC, int(tok[1]))
            elif tok[0] == "A" and uA is not None:
                stage_A(uA, sA, int(tok[1]))
            elif tok == "D" and uC is not None:
                stage_D(uC, o)
        while todo:
            stage_B(B_slot, todo.pop(0), NB)

    def finish_batch(b):
        ostage[b] = acc[b].astype(bf16)
        o_copy(b).start()

    wq0a = w_copy(wq_hbm, wq_v, 0, 0, 2)
    wq0b = w_copy(wq_hbm, wq_v, 1, 2, 2)
    wo0a = w_copy(woT_hbm, wo_v, 2, 0, 2)
    wo0b = w_copy(woT_hbm, wo_v, 3, 2, 2)
    x_copy(0).start()
    wq0a.start()
    wq0b.start()
    k_copy(0).start()
    x_copy(1).start()
    x_copy(2).start()
    v_copy(0).start()
    wo0a.start()
    wo0b.start()
    k_copy(1).start()
    x_copy(3).start()
    v_copy(1).start()
    for p in range(2, NP):
        k_copy(p).start()
    for p in range(2, NP - 1):
        v_copy(p).start()

    acc[...] = jnp.zeros_like(acc)
    x_copy(0).wait()
    stage_X(0)
    wq0a.wait()
    step(uQ=0, sQ=0)
    wq0b.wait()
    k_copy(0).wait()
    step(uQ=1, sQ=1, uA=0, sA=0)
    x_copy(1).wait()
    stage_X(1)
    step(uQ=2, sQ=0, uA=1, sA=1, B_slot=0)
    wo0a.wait()
    wo0b.wait()

    def w_group(gp):
        return _Multi([w_copy(wq_hbm, wq_v, 0, 4 * gp, 4), w_copy(woT_hbm, wo_v, 2, 4 * gp, 4)])

    def pair_iter(j, first_pass=False, last_pass=False):
        u0 = 2 * j
        k_copy(j + 1).wait()
        v_copy(j).wait()
        if first_pass:
            x_copy(j + 2).wait()
            stage_X(j + 2)
        step(uQ=u0 + 3, sQ=1, uA=u0 + 2, sA=0, B_slot=1, uC=u0, sC=0)
        k_copy(j + NP).start()
        v_copy(j - 1 + NP).start()
        if first_pass:
            @pl.when(j + 4 < B)
            def _():
                x_copy(j + 4).start()
        step(uQ=jnp.minimum(u0 + 4, n_units - 1), sQ=0, uA=u0 + 3, sA=1, B_slot=0, uC=u0 + 1, sC=1)
        if last_pass is True:
            finish_batch(j & (B - 1))
        elif last_pass is not False:
            @pl.when(last_pass)
            def _():
                finish_batch(j & (B - 1))

    w_group(1).start()

    def first_pass_body(j, c):
        pair_iter(j, first_pass=True)
        return c
    jax.lax.fori_loop(0, B - 2, first_pass_body, 0)

    def outer(gp, c):
        w_group(gp).wait()

        @pl.when(gp + 1 < GP)
        def _():
            w_group(gp + 1).start()

        def inner(i, c2):
            for k in range(UNROLL):
                j = gp * B - 2 + i * UNROLL + k
                pair_iter(j, last_pass=(j >= n_pairs - B))
            return c2
        jax.lax.fori_loop(0, B // UNROLL, inner, 0)
        return c
    jax.lax.fori_loop(1, GP, outer, 0)
    pair_iter(n_pairs - 2, last_pass=True)

    j = n_pairs - 1
    u0 = 2 * j
    v_copy(j).wait()
    step(B_slot=1, uC=u0, sC=0)
    step(uC=u0 + 1, sC=1)
    finish_batch(B - 1)
    for p in range(n_pairs, n_pairs + NP - 1):
        k_copy(p).wait()
    for p in range(n_pairs, n_pairs + NP - 2):
        v_copy(p).wait()
    pltpu.make_async_copy(ostage, outT_hbm, sem_o.at[0]).wait()


@jax.jit
def pallas_standalone__gqa_block_cached__near_ridge_kernel(x, k_cache, v_cache, wq, wo):
    B, Sq, D = x.shape
    _, Hkv, Sk, Dh = k_cache.shape
    Hq = wq.shape[1] // Dh
    assert Hq == 2 * Hkv and Hkv % 2 == 0
    GP = Hkv // 2
    xT = x.transpose(0, 2, 1)
    woT = wo.T
    k5 = k_cache.reshape(B, GP, 2, Sk, Dh)
    v5 = v_cache.reshape(B, GP, 2, Sk, Dh)
    kern = functools.partial(_kernel, scale=Dh ** -0.5 * LOG2E)
    bf16, f32, u32 = jnp.bfloat16, jnp.float32, jnp.uint32
    any_spec = pl.BlockSpec(memory_space=pl.ANY)
    V = pltpu.VMEM
    outT = pl.pallas_call(
        kern,
        in_specs=[any_spec] * 5,
        out_specs=any_spec,
        out_shape=jax.ShapeDtypeStruct((B, D, Sq), x.dtype),
        scratch_shapes=[
            V((B, D, Sq), bf16), V((B, Sq // 2, D), u32),
            V((Hq, D, Dh), bf16), V((Hq, D, Dh), bf16),
            V((NP, 2, Sk, Dh), bf16), V((NP, 2, Sk, Dh), bf16),
            V((Sq, Dh), u32), V((Sq, Dh), u32),
            V((2 * Sq, Sk), f32), V((2 * Sq, Sk), f32),
            V((2 * Sq, Dh), f32), V((2 * Sq, Dh), f32),
            V((Sq, Sk), u32), V((Sq, Sk), u32),
            V((2 * Sq, Dh), f32), V((2 * Sq, Dh), f32),
            V((2 * Sq, Dh), f32),
            V((B, D, Sq), f32), V((B, D, Sq), bf16),
            pltpu.SemaphoreType.DMA((4,)), pltpu.SemaphoreType.DMA((4,)),
            pltpu.SemaphoreType.DMA((NP,)), pltpu.SemaphoreType.DMA((NP,)),
            pltpu.SemaphoreType.DMA((1,)),
        ],
        compiler_params=pltpu.CompilerParams(vmem_limit_bytes=100 * 1024 * 1024,
                                             **({"flags": FLAGS} if FLAGS else {})),
    )(xT, k5, v5, wq, woT)
    return outT.transpose(0, 2, 1)
```

```python
import functools
import jax
import jax.numpy as jnp
import numpy as np
import jax.experimental.pallas as pl
import jax.experimental.pallas.tpu as pltpu

LOG2E = 1.4426950408889634
NP = 8
NP0 = 4
UNROLL = 4
UNROLL1 = 2
PEEL = 2
XAHEAD = 2
WSKIP = 1
NB = 8
NHA = 8
NHC = 2
ORDER = "B C0 B C1 B A0 A1 A2 A3 B A4 B A5 B D B A6 A7 B Q".split()


class _Multi:
    def __init__(self, copies):
        self.copies = copies

    def start(self):
        for c in self.copies:
            c.start()

    def wait(self):
        for c in self.copies:
            c.wait()


def _kernel(xT_hbm, k_hbm, v_hbm, wq_hbm, woT_hbm, outT_hbm,
            xT_v, x_scr, wq_v, wo_v, k_buf, v_buf,
            q0, q1, s0, s1, m0, m1, p0, p1, opart, oscr, acc, ostage,
            sem_x, sem_w, sem_k, sem_v, sem_o, *, scale):
    B, D, Sq = xT_hbm.shape
    _, GP, _, Sk, Dh = k_hbm.shape
    n_pairs = B * GP
    n_units = 2 * n_pairs
    assert UNROLL < NP and UNROLL1 < NP0 <= NP
    LB = B.bit_length() - 1
    assert B == 1 << LB
    f32, bf16, u32 = jnp.float32, jnp.bfloat16, jnp.uint32
    qs, ss, ms, ps = (q0, q1), (s0, s1), (m0, m1), (p0, p1)
    R = 2 * Sq
    NC = Sk // Dh
    HK = Sk // 2

    def batch_of(u):
        return (u >> 1) & (B - 1)

    def kvhead_of(u):
        return ((u >> (LB + 1)) << 1) | (u & 1)

    def k_copy(p):
        s = p & (NP - 1)
        pc = jnp.minimum(p, n_pairs - 1)
        return pltpu.make_async_copy(k_hbm.at[pc & (B - 1), pc >> LB], k_buf.at[s], sem_k.at[s])

    def v_copy(p):
        s = p & (NP - 1)
        pc = jnp.minimum(p, n_pairs - 1)
        return pltpu.make_async_copy(v_hbm.at[pc & (B - 1), pc >> LB], v_buf.at[s], sem_v.at[s])

    def w_copy(src, dst, which, h0, n):
        return _Multi([pltpu.make_async_copy(src.at[:, pl.ds(pl.multiple_of((h0 + i) * Dh, Dh), Dh)],
                                             dst.at[h0 + i], sem_w.at[which]) for i in range(n)])

    def x_copy(b, n=1):
        return pltpu.make_async_copy(xT_hbm.at[pl.ds(b, n)], xT_v.at[pl.ds(b, n)], sem_x.at[b])

    def o_copy(b):
        return pltpu.make_async_copy(ostage.at[b], outT_hbm.at[b], sem_o.at[0])

    def unpack(w):
        return pltpu.bitcast(w, bf16)

    def pack(v):
        return pltpu.bitcast(v, u32)

    def stage_X(b):
        x_scr[b] = pack(unpack(xT_v.bitcast(u32)[b]).T)

    def stage_Q(u, slot):
        g = kvhead_of(u)
        x = unpack(x_scr[batch_of(u)])
        wu = wq_v.bitcast(u32)
        w = jnp.concatenate([unpack(wu[2 * g]), unpack(wu[2 * g + 1])], axis=1)
        q = jnp.dot(x, w, preferred_element_type=f32)
        qs[slot][:Sq // 2, :] = pack(q[:, :Dh].astype(bf16))
        qs[slot][Sq // 2:, :] = pack(q[:, Dh:].astype(bf16))

    def stage_A(u, slot, h):
        HK = Sk // NHA
        k = unpack(k_buf.bitcast(u32)[(u >> 1) & (NP - 1), slot, h * (HK // 2):(h + 1) * (HK // 2), :])
        s = jax.lax.dot_general(unpack(qs[slot][...]), k, (((1,), (1,)), ((), ())),
                                preferred_element_type=f32)
        ss[slot][:, h * HK:(h + 1) * HK] = s
        mx = s[:, :Dh]
        for c in range(1, HK // Dh):
            mx = jnp.maximum(mx, s[:, c * Dh:(c + 1) * Dh])
        if h > 0:
            mx = jnp.maximum(mx, ms[slot][:R, :])
        if h == NHA - 1:
            mx = jnp.broadcast_to(jnp.max(mx, axis=-1, keepdims=True), (R, Dh))
        ms[slot][:R, :] = mx

    def stage_B(slot, i, n, z):
        rc = R // n
        rows = slice(i * rc, (i + 1) * rc)
        m = ms[slot][pl.ds(pl.multiple_of(i * rc + z, 8), rc), :]
        p = jnp.exp2((ss[slot][rows, :] - jnp.concatenate([m] * NC, axis=1)) * scale)
        l = p[:, :Dh]
        for c in range(1, NC):
            l = l + p[:, c * Dh:(c + 1) * Dh]
        l = jnp.sum(l, axis=-1, keepdims=True)
        r = pl.reciprocal(l, approx=True)
        r = r * (2.0 - l * r)
        ms[slot][R + i * rc:R + (i + 1) * rc, :] = jnp.broadcast_to(r, (rc, Dh))
        ps[slot][i * (rc // 2):(i + 1) * (rc // 2), :] = pack(p.astype(bf16))

    def stage_C(u, slot, h):
        HK = Sk // NHC
        v = unpack(v_buf.bitcast(u32)[(u >> 1) & (NP - 1), slot, h * (HK // 2):(h + 1) * (HK // 2), :])
        o = jnp.dot(unpack(ps[slot][:, h * HK:(h + 1) * HK]), v, preferred_element_type=f32)
        if h > 0:
            o = opart[...] + o
        if h < NHC - 1:
            opart[...] = o
            return
        oscr[...] = pack((o * ms[slot][R:, :]).astype(bf16))

    def stage_D(u):
        g = kvhead_of(u)
        b = batch_of(u)
        o = unpack(oscr[...])
        o2 = jnp.concatenate([o[:Sq], o[Sq:]], axis=1)
        wo_u = wo_v.bitcast(u32)
        w2 = jnp.concatenate([unpack(wo_u[2 * g]), unpack(wo_u[2 * g + 1])], axis=1)
        c = jax.lax.dot_general(w2, o2, (((1,), (1,)), ((), ())), preferred_element_type=f32)
        acc[b] += c

    def step(uQ=None, uA=None, B_slot=None, uC=None, sQ=0, sA=0, sC=0, z=0):
        todo = list(range(NB)) if B_slot is not None else []
        for tok in ORDER:
            if tok == "B":
                if todo:
                    stage_B(B_slot, todo.pop(0), NB, z)
            elif tok == "Q":
                if uQ is not None:
                    stage_Q(uQ, sQ)
            elif tok[0] == "C" and uC is not None:
                stage_C(uC, sC, int(tok[1]))
            elif tok[0] == "A" and uA is not None:
                stage_A(uA, sA, int(tok[1]))
            elif tok == "D" and uC is not None:
                stage_D(uC)
        while todo:
            stage_B(B_slot, todo.pop(0), NB, z)

    def finish_batch(b):
        ostage[b] = acc[b].astype(bf16)
        o_copy(b).start()

    wq0a = w_copy(wq_hbm, wq_v, 0, 0, 2)
    wq0b = w_copy(wq_hbm, wq_v, 1, 2, 2)
    wo0a = w_copy(woT_hbm, wo_v, 2, 0, 2)
    wo0b = w_copy(woT_hbm, wo_v, 3, 2, 2)
    def w_group(gp):
        return _Multi([w_copy(wq_hbm, wq_v, 0, 4 * gp, 4), w_copy(woT_hbm, wo_v, 2, 4 * gp, 4)])

    def start_all(*cs):
        for c in cs:
            c.start()

    start_all(x_copy(0), wq0a, wq0b, k_copy(0), x_copy(1))
    acc[...] = jnp.zeros_like(acc)
    x_copy(0).wait()
    stage_X(0)
    wq0a.wait()
    wq0b.wait()
    start_all(v_copy(0), wo0a, k_copy(1), x_copy(2), wo0b, x_copy(3))
    step(uQ=0, sQ=0)
    step(uQ=1, sQ=1)
    k_copy(0).wait()
    x_copy(1).wait()
    start_all(v_copy(1), k_copy(2))
    step(uA=0, sA=0)
    stage_X(1)
    step(uQ=2, sQ=0, uA=1, sA=1, B_slot=0)
    for t in range(4, 2 + PEEL + UNROLL1 + XAHEAD):
        x_copy(t).start()
    for t in range(3, NP0):
        v_copy(t - 1).start()
        k_copy(t).start()
    wo0a.wait()
    wo0b.wait()

    def pair_iters(j0, n, first_pass=False, last_pass=False, w_next=None, z=None):
        for k in range(n):
            k_copy(j0 + k + 1).wait()
            v_copy(j0 + k).wait()
            if first_pass:
                x_copy(j0 + k + 2).wait()
        for k in range(n):
            j = j0 + k
            if not isinstance(j, int):
                z = jnp.minimum(j, 0) * 8
            u0 = 2 * j
            if first_pass:
                stage_X(j + 2)
            step(uQ=u0 + 3, sQ=1, uA=u0 + 2, sA=0, B_slot=1, uC=u0, sC=0, z=z)
            if first_pass:
                ramp = B - 2 - (NP - NP0)
                ahead = NP0 + (max(j - ramp, 0) if isinstance(j, int) else jnp.maximum(j - ramp, 0))
                k_copy(j + ahead).start()
                v_copy(j + ahead - 1).start()

                @pl.when(j >= ramp)
                def _():
                    k_copy(j + ahead + 1).start()
                    v_copy(j + ahead).start()
            else:
                k_copy(j + NP).start()
                v_copy(j - 1 + NP).start()
            if first_pass:

                @pl.when((j >= PEEL) & (j + 2 + UNROLL1 + XAHEAD < B))
                def _():
                    x_copy(j + 2 + UNROLL1 + XAHEAD).start()
            if w_next is not None and k == 0:
                nblk = 4 if first_pass else min(4, B // UNROLL)

                @pl.when((w_next[1] >= 0) & (w_next[1] < nblk))
                def _():
                    nh = 4 // nblk
                    w_copy(wq_hbm, wq_v, 0, 4 * w_next[0] + w_next[1] * nh, nh).start()
                    w_copy(woT_hbm, wo_v, 2, 4 * w_next[0] + w_next[1] * nh, nh).start()
            if isinstance(j, int):
                uq = u0 + 4 if u0 + 4 < n_units else None
            else:
                assert not (last_pass and n == 1)
                uq = u0 + 4
            step(uQ=uq, sQ=0, uA=u0 + 3, sA=1, B_slot=0, uC=u0 + 1, sC=1, z=z)
            if last_pass:
                bb = j & (B - 1)
                ostage[bb] = acc[bb].astype(bf16)

                @pl.when(j >= n_pairs - B)
                def _():
                    o_copy(bb).start()

    def peel_body(j, c):
        pair_iters(j, 1, first_pass=True)
        return c
    jax.lax.fori_loop(0, PEEL, peel_body, 0)

    def first_pass_body(i, c):
        pair_iters(PEEL + i * UNROLL1, UNROLL1, first_pass=True, w_next=(1, i - WSKIP))
        return c
    assert (B - 2 - PEEL) % UNROLL1 == 0 and WSKIP + 4 <= (B - 2 - PEEL) // UNROLL1
    jax.lax.fori_loop(0, (B - 2 - PEEL) // UNROLL1, first_pass_body, 0)

    def outer(gp, c):
        w_group(gp).wait()

        def inner(i, c2):
            pair_iters(gp * B - 2 + i * UNROLL, UNROLL, w_next=(gp + 1, i))
            return c2
        jax.lax.fori_loop(0, B // UNROLL, inner, 0)
        return c
    jax.lax.fori_loop(1, GP - 1, outer, 0)

    w_group(GP - 1).wait()

    def last_pass_body(i, c):
        pair_iters((GP - 1) * B - 2 + i * UNROLL, UNROLL, last_pass=True)
        return jnp.minimum(i, 0) * 8
    zero = jax.lax.fori_loop(0, B // UNROLL, last_pass_body, np.int32(0))
    v_copy(n_pairs - 1).wait()
    pair_iters(n_pairs - 2, 1, last_pass=True, z=zero)

    j = n_pairs - 1
    u0 = 2 * j
    step(B_slot=1, uC=u0, sC=0, z=zero)
    step(uC=u0 + 1, sC=1)
    finish_batch(B - 1)
    for p in range(n_pairs, n_pairs + NP - 1):
        k_copy(p).wait()
    for p in range(n_pairs, n_pairs + NP - 2):
        v_copy(p).wait()
    pltpu.make_async_copy(ostage, outT_hbm, sem_o.at[0]).wait()


@jax.jit
def pallas_standalone__gqa_block_cached__near_ridge_kernel(x, k_cache, v_cache, wq, wo):
    B, Sq, D = x.shape
    _, Hkv, Sk, Dh = k_cache.shape
    Hq = wq.shape[1] // Dh
    assert Hq == 2 * Hkv and Hkv % 2 == 0
    GP = Hkv // 2
    xT = x.transpose(0, 2, 1)
    woT = wo.T
    k5 = k_cache.reshape(B, GP, 2, Sk, Dh)
    v5 = v_cache.reshape(B, GP, 2, Sk, Dh)
    kern = functools.partial(_kernel, scale=Dh ** -0.5 * LOG2E)
    bf16, f32, u32 = jnp.bfloat16, jnp.float32, jnp.uint32
    any_spec = pl.BlockSpec(memory_space=pl.ANY)
    V = pltpu.VMEM
    outT = pl.pallas_call(
        kern,
        in_specs=[any_spec] * 5,
        out_specs=any_spec,
        out_shape=jax.ShapeDtypeStruct((B, D, Sq), x.dtype),
        scratch_shapes=[
            V((B, D, Sq), bf16), V((B, Sq // 2, D), u32),
            V((Hq, D, Dh), bf16), V((Hq, D, Dh), bf16),
            V((NP, 2, Sk, Dh), bf16), V((NP, 2, Sk, Dh), bf16),
            V((Sq, Dh), u32), V((Sq, Dh), u32),
            V((2 * Sq, Sk), f32), V((2 * Sq, Sk), f32),
            V((4 * Sq, Dh), f32), V((4 * Sq, Dh), f32),
            V((Sq, Sk), u32), V((Sq, Sk), u32),
            V((2 * Sq, Dh), f32), V((Sq, Dh), u32),
            V((B, D, Sq), f32), V((B, D, Sq), bf16),
            pltpu.SemaphoreType.DMA((B,)), pltpu.SemaphoreType.DMA((4,)),
            pltpu.SemaphoreType.DMA((NP,)), pltpu.SemaphoreType.DMA((NP,)),
            pltpu.SemaphoreType.DMA((1,)),
        ],
        compiler_params=pltpu.CompilerParams(vmem_limit_bytes=100 * 1024 * 1024),
    )(xT, k5, v5, wq, woT)
    return outT.transpose(0, 2, 1)
```
